```python
import jax
import jax.numpy as jnp

def _softmax(x, axis=-1):
    return jax.nn.softmax(x, axis=axis)
def _gelu(x):
    return jax.nn.gelu(x, approximate=True)
def _silu(x):
    return jax.nn.silu(x)
def _sigmoid(x):
    return jax.nn.sigmoid(x)
def _layernorm(x, axis=-1, eps=1e-5):
    m = jnp.mean(x, axis=axis, keepdims=True)
    v = jnp.var(x, axis=axis, keepdims=True)
    return (x - m) / jnp.sqrt(v + eps)
def _scatter_add(tgt, idx, src, axis=0):
    return tgt.at[idx].add(src)
def _segment_sum(src, seg, n):
    return jax.ops.segment_sum(src, seg, n)
class _Rng:
    def __init__(self, key):
        self._k = key
    def _next(self):
        self._k, sub = jax.random.split(self._k)
        return sub
    def normal(self, shape):
        return jax.random.normal(self._next(), shape, dtype=jnp.bfloat16)
    def randint(self, lo, hi, shape):
        return jax.random.randint(self._next(), shape, lo, hi, dtype=jnp.int32)
    def uniform(self, shape, lo=0.0, hi=1.0):
        return jax.random.uniform(self._next(), shape, jnp.bfloat16, lo, hi)
    def permutation(self, n):
        return jax.random.permutation(self._next(), n)


kernel_name = 'concat_heads__gqa_block_cached__compressed_kv_cla__decode'

def setup_inputs():
    _rng = _Rng(jax.random.key(int.from_bytes(__import__("os").urandom(4), "little")))
    _w = (lambda a: (lambda t: t.astype(jnp.bfloat16) if jnp.issubdtype(t.dtype, jnp.floating) else t)(jnp.asarray(a)))
    def _A_setup():
        B, Sq, D = 2, 1, 512
        Hq, Hkv, Sk, Dh = 32, 32, 8192, 128
        assert Hq % Hkv == 0, (Hq, Hkv)
        return {
            "x": _w((lambda *s: _rng.normal(s) * 0.05)(B, Sq, D)),
            "k_cache": _w((lambda *s: _rng.normal(s) * 0.05)(B, Hkv, Sk, Dh)),
            "v_cache": _w((lambda *s: _rng.normal(s) * 0.05)(B, Hkv, Sk, Dh)),
            "wq": _w((lambda *s: _rng.normal(s) * 0.05)(D, Hq * Dh) * (D ** -0.5)),
            "wo": _w((lambda *s: _rng.normal(s) * 0.05)(Hq * Dh, D) * ((Hq * Dh) ** -0.5)),
        }
    _A_in = _A_setup()

    def _B_setup():
        B, H, Sq, Sk, D, M = 2, 32, 1, 8192, 128, 512
        Dc = 4 * D
        return {
            "x": _w((lambda *s: _rng.normal(s) * 0.05)(B, Sq, M)),
            "c_kv": _w((lambda *s: _rng.normal(s) * 0.05)(B, Sk, Dc)),
            "w_q": _w((lambda *s: _rng.normal(s) * 0.05)(M, H, D) * (M ** -0.5)),
            "w_uk": _w((lambda *s: _rng.normal(s) * 0.05)(Dc, H, D) * (Dc ** -0.5)),
            "w_uv": _w((lambda *s: _rng.normal(s) * 0.05)(Dc, H, D) * (Dc ** -0.5)),
            "w_o": _w((lambda *s: _rng.normal(s) * 0.05)(H, D, M) * ((H * D) ** -0.5)),
        }
    _B_in = _B_setup()

    return {
        "A_x": _A_in["x"],
        "A_k_cache": _A_in["k_cache"],
        "A_v_cache": _A_in["v_cache"],
        "A_wq": _A_in["wq"],
        "A_wo": _A_in["wo"],
        "B_x": _B_in["x"],
        "B_c_kv": _B_in["c_kv"],
        "B_w_q": _B_in["w_q"],
        "B_w_uk": _B_in["w_uk"],
        "B_w_uv": _B_in["w_uv"],
        "B_w_o": _B_in["w_o"],
    }

def reference(A_x, A_k_cache, A_v_cache, A_wq, A_wo, B_x, B_c_kv, B_w_q, B_w_uk, B_w_uv, B_w_o):
    def _A_ref(x, k_cache, v_cache, wq, wo):
        B, Sq, D = x.shape
        Hq, Dh = 32, 128
        Hkv = k_cache.shape[1]
        rep = Hq // Hkv
        q = (lambda x, *d: x.transpose(*d))((x @ wq).reshape(B, Sq, Hq, Dh), 0, 2, 1, 3)
        k = jnp.repeat(k_cache, rep, axis=1)
        v = jnp.repeat(v_cache, rep, axis=1)
        scores = jnp.einsum("bhqd,bhkd->bhqk", q, k) * (Dh ** -0.5)
        p = _softmax(scores, axis=-1)
        o = jnp.einsum("bhqk,bhkd->bhqd", p, v)
        return (lambda x, *d: x.transpose(*d))(o, 0, 2, 1, 3).reshape(B, Sq, Hq * Dh) @ wo

    def _B_ref(x, c_kv, w_q, w_uk, w_uv, w_o):
        B, Sq, M = x.shape[0], x.shape[1], x.shape[2]
        Sk = c_kv.shape[1]
        H, D = w_q.shape[1], w_q.shape[2]
        q = jnp.einsum("bqm,mhd->bhqd", x, w_q)
        k = jnp.einsum("bkc,chd->bhkd", c_kv, w_uk)
        v = jnp.einsum("bkc,chd->bhkd", c_kv, w_uv)
        scores = jnp.einsum("bhqd,bhkd->bhqk", q, k) * (D ** -0.5)
        off = Sk - Sq
        qi = jnp.arange(Sq)[:, None]
        kj = jnp.arange(Sk)[None, :]
        cmask = kj <= (qi + off)
        scores = jnp.where(cmask[None, None], scores, -1e9)
        p = _softmax(scores, axis=-1)
        ctx = jnp.einsum("bhqk,bhkd->bhqd", p, v)
        return jnp.einsum("bhqd,hdm->bqm", ctx, w_o)

    a = _A_ref(A_x, A_k_cache, A_v_cache, A_wq, A_wo)
    b = _B_ref(B_x, B_c_kv, B_w_q, B_w_uk, B_w_uv, B_w_o)
    return jnp.concatenate([a, b], axis=-1)
```

```python
import functools
import math

import jax
import jax.numpy as jnp
from jax import lax
import jax.experimental.pallas as pl
import jax.experimental.pallas.tpu as pltpu

NB = 2
H = 32
SK = 8192
DH = 128
DM = 512
DC = 512

R = 4
CH = 128
NCH = SK // CH
XPI = 16
BCH = 1024

W1_ITERS = 128 // XPI
CKV_ITERS = 256 // XPI
W2_ITERS = 128 // XPI
IT_CKV0 = W1_ITERS
IT_W20 = IT_CKV0 + CKV_ITERS
IT_WEND = IT_W20 + W2_ITERS
IT_BQ = IT_CKV0 + R
IT_BATT = IT_W20 + R
IT_BFIN = max(IT_WEND + R, IT_BATT + 3)

S_XA, S_XB, S_WQA, S_WOA, S_WQB, S_WUK, S_WUV, S_WOB, S_CKV0, S_K0 = range(8 + 2)
S_XA, S_XB, S_WQA, S_WOA, S_WQB, S_WUK, S_WUV, S_WOB = range(8)
S_CKV0 = 8
S_K0 = 10
S_V0 = S_K0 + R
NSEM = S_V0 + R

LOG2E = math.log2(math.e)


def _rows2(r0, r1, n):
    shape = (n, r0.shape[-1])
    row = lax.broadcasted_iota(jnp.int32, shape, 0)
    return jnp.where(row == 0, jnp.broadcast_to(r0, shape),
                     jnp.where(row == 1, jnp.broadcast_to(r1, shape), 0.0))


def _split_pair(w_u32):
    lo = lax.bitcast_convert_type(w_u32 << 16, jnp.float32)
    hi = lax.bitcast_convert_type(w_u32 & jnp.uint32(0xFFFF0000), jnp.float32)
    return lo.astype(jnp.bfloat16), hi.astype(jnp.bfloat16)


def _kernel(xa_hbm, k_hbm, v_hbm, wqa_hbm, woa_hbm,
            xb_hbm, ckv_hbm, wqb_hbm, wuk_hbm, wuv_hbm, wob_hbm,
            out_ref,
            xa_v, xb_v, kbuf, vbuf, wqa_v, woa_v, ckv_v, wqb_v, wuk_v, wuv_v, wob_v,
            qa_ref, acca_ref, ql_ref, sb_ref, cl_ref, accb_ref, sems):

    def kv_start(i, slot):
        b = i // H
        h = i % H
        for c in range(NCH):
            rows = pl.ds(c * CH, CH)
            pltpu.make_async_copy(k_hbm.at[b, h, rows, :], kbuf.at[slot, rows, :],
                                  sems.at[S_K0 + slot]).start(priority=0)
            pltpu.make_async_copy(v_hbm.at[b, h, rows, :], vbuf.at[slot, rows, :],
                                  sems.at[S_V0 + slot]).start(priority=1)

    def k_wait(slot):
        pltpu.make_async_copy(k_hbm.at[0, 0], kbuf.at[slot], sems.at[S_K0 + slot]).wait()

    def v_wait(slot):
        pltpu.make_async_copy(v_hbm.at[0, 0], vbuf.at[slot], sems.at[S_V0 + slot]).wait()

    def w3_src(w_hbm):
        return w_hbm.bitcast(jnp.uint32)

    def w3_dst(w_v):
        return w_v.reshape(DM, H // 2, DH)

    def w3_chunk(w_hbm, w_v, sem, c, prio):
        rows = pl.ds(pl.multiple_of(c * 4, 4), 4)
        pltpu.make_async_copy(w3_src(w_hbm).at[rows], w3_dst(w_v).at[rows],
                              sems.at[sem]).start(priority=prio)

    def w3_wait(w_hbm, w_v, sem):
        pltpu.make_async_copy(w3_src(w_hbm), w3_dst(w_v), sems.at[sem]).wait()

    pltpu.make_async_copy(xa_hbm, xa_v, sems.at[S_XA]).start(priority=0)
    pltpu.make_async_copy(xb_hbm, xb_v, sems.at[S_XB]).start(priority=1)
    for c in range(128):
        r, cc = divmod(c, 4)
        rs, cs = pl.ds(r * 16, 16), pl.ds(cc * 1024, 1024)
        pltpu.make_async_copy(wqa_hbm.at[rs, cs], wqa_v.at[rs, cs],
                              sems.at[S_WQA]).start(priority=0)
        rs = pl.ds(c * 32, 32)
        pltpu.make_async_copy(woa_hbm.at[rs, :], woa_v.at[rs, :],
                              sems.at[S_WOA]).start(priority=1)
    for s in range(R):
        kv_start(s, s)

    pltpu.make_async_copy(xa_hbm, xa_v, sems.at[S_XA]).wait()
    pltpu.make_async_copy(wqa_hbm, wqa_v, sems.at[S_WQA]).wait()
    xa = _rows2(xa_v[0].astype(jnp.float32), xa_v[1].astype(jnp.float32), 16)
    qa = jnp.dot(xa.astype(jnp.bfloat16), wqa_v[...],
                 preferred_element_type=jnp.float32)
    qa = qa.astype(jnp.bfloat16).astype(jnp.float32)
    for b in range(NB):
        for h in range(H):
            qa_ref[pl.ds(b * H + h, 1), :] = qa[b:b + 1, h * DH:(h + 1) * DH]
    acca_ref[...] = jnp.zeros(acca_ref.shape, jnp.float32)
    accb_ref[...] = jnp.zeros(accb_ref.shape, jnp.float32)
    pltpu.make_async_copy(woa_hbm, woa_v, sems.at[S_WOA]).wait()

    sc2 = jnp.float32(DH ** -0.5 * LOG2E)

    def b_queries():
        pltpu.make_async_copy(xb_hbm, xb_v, sems.at[S_XB]).wait()
        w3_wait(wqb_hbm, wqb_v, S_WQB)
        w3_wait(wuk_hbm, wuk_v, S_WUK)
        xb = _rows2(xb_v[0].astype(jnp.float32), xb_v[1].astype(jnp.float32), 16)
        xb = xb.astype(jnp.bfloat16)

        def pair(j, carry):
            wq2 = _split_pair(wqb_v[pl.ds(j, DM, stride=H // 2), :])
            wk2 = _split_pair(wuk_v[pl.ds(j, DC, stride=H // 2), :])
            for hh in range(2):
                h = 2 * j + hh
                q = jnp.dot(xb, wq2[hh], preferred_element_type=jnp.float32)
                ql = lax.dot_general(q.astype(jnp.bfloat16), wk2[hh],
                                     (((1,), (1,)), ((), ())),
                                     preferred_element_type=jnp.float32)
                ql_ref[pl.ds(h, 1), :] = ql[0:1, :]
                ql_ref[pl.ds(H + h, 1), :] = ql[1:2, :]
            return carry

        lax.fori_loop(0, H // 2, pair, 0)

    def b_attention(b):
        pltpu.make_async_copy(ckv_hbm.at[0], ckv_v.at[0], sems.at[S_CKV0 + b]).wait()
        r0 = pl.multiple_of(b * H, H)
        ql = ql_ref[pl.ds(r0, H), :].astype(jnp.bfloat16)

        def scores(j, m):
            k0 = pl.multiple_of(j * BCH, BCH)
            c = ckv_v[b, pl.ds(k0, BCH), :]
            s = lax.dot_general(ql, c, (((1,), (1,)), ((), ())),
                                preferred_element_type=jnp.float32)
            sb_ref[:, pl.ds(k0, BCH)] = s
            return jnp.maximum(m, jnp.max(s, axis=-1, keepdims=True))

        m = lax.fori_loop(0, SK // BCH, scores,
                          jnp.full((H, 1), -jnp.inf, jnp.float32))

        def values(j, carry):
            l, acc = carry
            k0 = pl.multiple_of(j * BCH, BCH)
            p = jnp.exp2((sb_ref[:, pl.ds(k0, BCH)] - m) * sc2)
            l = l + jnp.sum(p, axis=-1, keepdims=True)
            c = ckv_v[b, pl.ds(k0, BCH), :]
            acc = acc + jnp.dot(p.astype(jnp.bfloat16), c,
                                preferred_element_type=jnp.float32)
            return l, acc

        l, acc = lax.fori_loop(0, SK // BCH, values,
                               (jnp.zeros((H, 1), jnp.float32),
                                jnp.zeros((H, DC), jnp.float32)))
        cl_ref[pl.ds(r0, H), :] = acc / l

    def b_finish():
        w3_wait(wuv_hbm, wuv_v, S_WUV)
        pltpu.make_async_copy(wob_hbm, wob_v, sems.at[S_WOB]).wait()

        def pair(j, acc):
            wv2 = _split_pair(wuv_v[pl.ds(j, DC, stride=H // 2), :])
            for hh in range(2):
                h = 2 * j + hh
                cl = _rows2(cl_ref[pl.ds(h, 1), :], cl_ref[pl.ds(H + h, 1), :], 16)
                ctx = jnp.dot(cl.astype(jnp.bfloat16), wv2[hh],
                              preferred_element_type=jnp.float32)
                acc = acc + jnp.dot(ctx.astype(jnp.bfloat16), wob_v[h],
                                    preferred_element_type=jnp.float32)
            return acc

        acc = lax.fori_loop(0, H // 2, pair, jnp.zeros((16, DM), jnp.float32))
        accb_ref[...] = acc[0:8, :]

    def step(i, carry):
        slot = i % R
        b = i // H
        h = i % H

        k_wait(slot)
        q = jnp.broadcast_to(qa_ref[pl.ds(i, 1), :], (8, DH)).astype(jnp.bfloat16)
        s = lax.dot_general(q, kbuf[slot], (((1,), (1,)), ((), ())),
                            preferred_element_type=jnp.float32)
        m = jnp.max(s, axis=-1, keepdims=True)
        p = jnp.exp2((s - m) * sc2)
        l = jnp.sum(p, axis=-1, keepdims=True)
        v_wait(slot)
        o = jnp.dot(p.astype(jnp.bfloat16), vbuf[slot],
                    preferred_element_type=jnp.float32)

        @pl.when(i + R < NB * H)
        def _():
            kv_start(i + R, slot)

        @pl.when(i < IT_CKV0)
        def _():
            for c in range(XPI):
                w3_chunk(wqb_hbm, wqb_v, S_WQB, i * XPI + c, 0)
                w3_chunk(wuk_hbm, wuk_v, S_WUK, i * XPI + c, 1)

        @pl.when(jnp.logical_and(i >= IT_CKV0, i < IT_W20))
        def _():
            for c in range(XPI):
                rows = pl.ds(pl.multiple_of(((i - IT_CKV0) * XPI + c) * 32, 32), 32)
                for bb in range(NB):
                    pltpu.make_async_copy(ckv_hbm.at[bb, rows, :], ckv_v.at[bb, rows, :],
                                          sems.at[S_CKV0 + bb]).start(priority=bb)

        @pl.when(jnp.logical_and(i >= IT_W20, i < IT_WEND))
        def _():
            for c in range(XPI):
                cc = (i - IT_W20) * XPI + c
                w3_chunk(wuv_hbm, wuv_v, S_WUV, cc, 0)
                rows = pl.ds(pl.multiple_of((cc % 4) * 32, 32), 32)
                pltpu.make_async_copy(wob_hbm.at[cc // 4, rows, :], wob_v.at[cc // 4, rows, :],
                                      sems.at[S_WOB]).start(priority=1)

        o = (o / l).astype(jnp.bfloat16)
        w0 = pl.multiple_of(h * DH, DH)
        acca_ref[b] += jnp.dot(o, woa_v[pl.ds(w0, DH), :],
                               preferred_element_type=jnp.float32)

        @pl.when(i == IT_BQ)
        def _():
            b_queries()

        @pl.when(jnp.logical_or(i == IT_BATT, i == IT_BATT + 2))
        def _():
            b_attention((i - IT_BATT) // 2)

        @pl.when(i == IT_BFIN)
        def _():
            b_finish()

        return carry

    lax.fori_loop(0, NB * H, step, 0)

    for b in range(NB):
        out_ref[b, :, 0:DM] = acca_ref[b, 0:1, :].astype(out_ref.dtype)
        out_ref[b, :, DM:2 * DM] = accb_ref[b:b + 1, :].astype(out_ref.dtype)


@jax.jit
def pallas_concat_heads__gqa_block_cached__compressed_kv_cla__decode_kernel(
    A_x: jax.Array,
    A_k_cache: jax.Array,
    A_v_cache: jax.Array,
    A_wq: jax.Array,
    A_wo: jax.Array,
    B_x: jax.Array,
    B_c_kv: jax.Array,
    B_w_q: jax.Array,
    B_w_uk: jax.Array,
    B_w_uv: jax.Array,
    B_w_o: jax.Array,
):
    assert A_x.shape == (NB, 1, DM) and B_x.shape == (NB, 1, DM)
    assert A_k_cache.shape == (NB, H, SK, DH) and A_v_cache.shape == (NB, H, SK, DH)
    assert B_c_kv.shape == (NB, SK, DC)
    bf16, f32, u32 = jnp.bfloat16, jnp.float32, jnp.uint32
    any_spec = pl.BlockSpec(memory_space=pl.ANY)
    return pl.pallas_call(
        _kernel,
        out_shape=jax.ShapeDtypeStruct((NB, 1, 2 * DM), bf16),
        in_specs=[any_spec] * 11,
        out_specs=pl.BlockSpec(memory_space=pltpu.VMEM),
        scratch_shapes=[
            pltpu.VMEM((NB, 1, DM), bf16),
            pltpu.VMEM((NB, 1, DM), bf16),
            pltpu.VMEM((R, SK, DH), bf16),
            pltpu.VMEM((R, SK, DH), bf16),
            pltpu.VMEM((DM, H * DH), bf16),
            pltpu.VMEM((H * DH, DM), bf16),
            pltpu.VMEM((NB, SK, DC), bf16),
            pltpu.VMEM((DM * H // 2, DH), u32),
            pltpu.VMEM((DC * H // 2, DH), u32),
            pltpu.VMEM((DC * H // 2, DH), u32),
            pltpu.VMEM((H, DH, DM), bf16),
            pltpu.VMEM((NB * H, DH), f32),
            pltpu.VMEM((NB, 8, DM), f32),
            pltpu.VMEM((NB * H, DC), f32),
            pltpu.VMEM((H, SK), f32),
            pltpu.VMEM((NB * H, DC), f32),
            pltpu.VMEM((8, DM), f32),
            pltpu.SemaphoreType.DMA((NSEM,)),
        ],
        compiler_params=pltpu.CompilerParams(vmem_limit_bytes=100 * 1024 * 1024),
    )(A_x, A_k_cache, A_v_cache, A_wq, A_wo, B_x, B_c_kv, B_w_q, B_w_uk, B_w_uv, B_w_o)
```

```python
import math

import jax
import jax.numpy as jnp
from jax import lax
import jax.experimental.pallas as pl
import jax.experimental.pallas.tpu as pltpu

NB = 2
H = 32
SK = 8192
DH = 128
DM = 512
DC = 512

R = 2
NSTR = 4
CH = 64
NCH = (SK // 2) // CH
XPI = 16
XSTR = 4
BCH = 1024

W1_ITERS = 128 // XPI
CKV_ITERS = 256 // XPI
W2_ITERS = 128 // XPI
IT_CKV0 = W1_ITERS
IT_W20 = IT_CKV0 + CKV_ITERS
IT_WEND = IT_W20 + W2_ITERS
NBCH = SK // BCH
IT_P1 = IT_CKV0 + 1
IT_P2 = max(IT_P1 + H // 2, IT_W20 + 1)
IT_P3 = IT_P2 + NBCH
IT_P4 = max(IT_P3 + NBCH, IT_WEND + 1)
assert IT_P4 + H // 2 <= NB * H

S_XA, S_XB, S_WQA, S_WOA, S_WQB, S_WUK, S_WUV, S_WOB = range(8)
S_CKV0 = 8
S_K0 = 10
S_V0 = S_K0 + R
NSEM = S_V0 + R

LOG2E = math.log2(math.e)


def _rows2(r0, r1, n):
    shape = (n, r0.shape[-1])
    row = lax.broadcasted_iota(jnp.int32, shape, 0)
    return jnp.where(row == 0, jnp.broadcast_to(r0, shape),
                     jnp.where(row == 1, jnp.broadcast_to(r1, shape), 0.0))


def _split_pair(w_u32):
    lo = lax.bitcast_convert_type(w_u32 << 16, jnp.float32)
    hi = lax.bitcast_convert_type(w_u32 & jnp.uint32(0xFFFF0000), jnp.float32)
    return lo.astype(jnp.bfloat16), hi.astype(jnp.bfloat16)


def _stream_order(n, nstr):
    per = n // nstr
    return [s * per + j for j in range(per) for s in range(nstr)]


def _kernel(xa_hbm, k_hbm, v_hbm, wqa_hbm, woa_hbm,
            xb_hbm, ckv_hbm, wqb_hbm, wuk_hbm, wuv_hbm, wob_hbm,
            out_ref,
            xa_v, xb_v, kbuf, vbuf, wqa_v, woa_v, ckv_v, wqb_v, wuk_v, wuv_v, wob_v,
            qa_ref, acca_ref, ql_ref, sb_ref, mb_ref, lb_ref, cl_ref, accb_ref, sems):
    u32, f32, bf16 = jnp.uint32, jnp.float32, jnp.bfloat16
    NT = (((1,), (1,)), ((), ()))

    k32 = k_hbm.bitcast(u32)
    v32 = v_hbm.bitcast(u32)

    def kv_start(i, slot):
        b = i // H
        h = i % H
        for c in _stream_order(NCH, NSTR):
            rows = pl.ds(c * CH, CH)
            pltpu.make_async_copy(k32.at[b, h, rows, :], kbuf.at[slot, rows, :],
                                  sems.at[S_K0 + slot]).start(priority=0)
            pltpu.make_async_copy(v32.at[b, h, rows, :], vbuf.at[slot, rows, :],
                                  sems.at[S_V0 + slot]).start(priority=1)

    def k_wait(slot):
        pltpu.make_async_copy(k32.at[0, 0], kbuf.at[slot], sems.at[S_K0 + slot]).wait()

    def v_wait(slot):
        pltpu.make_async_copy(v32.at[0, 0], vbuf.at[slot], sems.at[S_V0 + slot]).wait()

    def w3_src(w_hbm):
        return w_hbm.bitcast(u32)

    def w3_dst(w_v):
        return w_v.reshape(DM, H // 2, DH)

    def w3_chunk(w_hbm, w_v, sem, c, prio):
        rows = pl.ds(pl.multiple_of(c * 4, 4), 4)
        pltpu.make_async_copy(w3_src(w_hbm).at[rows], w3_dst(w_v).at[rows],
                              sems.at[sem]).start(priority=prio)

    def w3_wait(w_hbm, w_v, sem):
        pltpu.make_async_copy(w3_src(w_hbm), w3_dst(w_v), sems.at[sem]).wait()

    def xchunks(it, total):
        per = total // XSTR
        n = XPI // XSTR
        return [s * per + it * n + j for j in range(n) for s in range(XSTR)]

    pltpu.make_async_copy(xa_hbm, xa_v, sems.at[S_XA]).start(priority=0)
    pltpu.make_async_copy(xb_hbm, xb_v, sems.at[S_XB]).start(priority=1)
    for c in _stream_order(128, XSTR):
        r, cc = divmod(c, 4)
        rs, cs = pl.ds(r * 16, 16), pl.ds(cc * 1024, 1024)
        pltpu.make_async_copy(wqa_hbm.at[rs, cs], wqa_v.at[rs, cs],
                              sems.at[S_WQA]).start(priority=0)
        rs = pl.ds(c * 32, 32)
        pltpu.make_async_copy(woa_hbm.at[rs, :], woa_v.at[rs, :],
                              sems.at[S_WOA]).start(priority=1)
    kv_start(0, 0)

    pltpu.make_async_copy(xa_hbm, xa_v, sems.at[S_XA]).wait()
    pltpu.make_async_copy(wqa_hbm, wqa_v, sems.at[S_WQA]).wait()
    xa = xa_v[...].astype(f32)
    xa = _rows2(xa[0:1], xa[1:2], 16)
    qa = jnp.dot(xa.astype(bf16), wqa_v[...], preferred_element_type=f32)
    qa = qa.astype(bf16).astype(f32)
    for b in range(NB):
        for h in range(H):
            qa_ref[pl.ds(b * H + h, 1), :] = qa[b:b + 1, h * DH:(h + 1) * DH]

    for s in range(1, R):
        kv_start(s, s)

    acca_ref[...] = jnp.zeros(acca_ref.shape, f32)
    accb_ref[...] = jnp.zeros(accb_ref.shape, f32)
    mb_ref[...] = jnp.full(mb_ref.shape, -jnp.inf, f32)
    lb_ref[...] = jnp.zeros(lb_ref.shape, f32)
    cl_ref[...] = jnp.zeros(cl_ref.shape, f32)
    pltpu.make_async_copy(woa_hbm, woa_v, sems.at[S_WOA]).wait()

    sc2 = DH ** -0.5 * LOG2E

    def b_query_piece(j):
        xb = xb_v[...].astype(f32)
        xb = _rows2(xb[0:1], xb[1:2], 16).astype(bf16)
        wq2 = _split_pair(wqb_v[pl.ds(j, DM, stride=H // 2), :])
        wk2 = _split_pair(wuk_v[pl.ds(j, DC, stride=H // 2), :])
        for hh in range(2):
            h = 2 * j + hh
            q = jnp.dot(xb, wq2[hh], preferred_element_type=f32)
            ql = lax.dot_general(q.astype(bf16), wk2[hh], NT,
                                 preferred_element_type=f32)
            ql_ref[pl.ds(h, 1), :] = ql[0:1, :]
            ql_ref[pl.ds(H + h, 1), :] = ql[1:2, :]

    def b_score_piece(b, j):
        k0 = pl.multiple_of(j * BCH, BCH)
        ql = ql_ref[b * H:(b + 1) * H, :].astype(bf16)
        s = lax.dot_general(ql, ckv_v[b, pl.ds(k0, BCH), :], NT,
                            preferred_element_type=f32)
        sb_ref[b * H:(b + 1) * H, pl.ds(k0, BCH)] = s
        m = jnp.max(s, axis=-1, keepdims=True)
        mb_ref[b * H:(b + 1) * H, :] = jnp.maximum(mb_ref[b * H:(b + 1) * H, :], m)

    def b_value_piece(b, j):
        k0 = pl.multiple_of(j * BCH, BCH)
        rows = slice(b * H, (b + 1) * H)
        m = mb_ref[rows, 0:1]
        p = jnp.exp2((sb_ref[rows, pl.ds(k0, BCH)] - m) * sc2)
        lb_ref[rows, :] += jnp.sum(p, axis=-1, keepdims=True)
        cl_ref[rows, :] += jnp.dot(p.astype(bf16), ckv_v[b, pl.ds(k0, BCH), :],
                                   preferred_element_type=f32)

    def b_out_piece(j):
        wv2 = _split_pair(wuv_v[pl.ds(j, DC, stride=H // 2), :])
        acc = accb_ref[...]
        for hh in range(2):
            h = 2 * j + hh
            cl = _rows2(cl_ref[pl.ds(h, 1), :], cl_ref[pl.ds(H + h, 1), :], 16)
            ctx = jnp.dot(cl.astype(bf16), wv2[hh], preferred_element_type=f32)
            acc = acc + jnp.dot(ctx.astype(bf16), wob_v[h],
                                preferred_element_type=f32)[0:8]
        accb_ref[...] = acc

    def step(i, carry):
        slot = i % R
        b = i // H
        h = i % H

        k_wait(slot)
        q = jnp.broadcast_to(qa_ref[pl.ds(i, 1), :], (8, DH)).astype(bf16)
        kk = pltpu.bitcast(kbuf[slot], bf16)
        s = lax.dot_general(q, kk, NT, preferred_element_type=f32)
        m = jnp.max(s, axis=-1, keepdims=True)
        p = jnp.exp2((s - m) * sc2)
        l = jnp.sum(p, axis=-1, keepdims=True)
        v_wait(slot)
        vv = pltpu.bitcast(vbuf[slot], bf16)
        o = jnp.dot(p.astype(bf16), vv, preferred_element_type=f32)
        o = (o / l).astype(bf16)
        w0 = pl.multiple_of(h * DH, DH)
        acca_ref[b] += jnp.dot(o, woa_v[pl.ds(w0, DH), :], preferred_element_type=f32)

        @pl.when(i + R < NB * H)
        def _():
            kv_start(i + R, slot)

        @pl.when(i < IT_CKV0)
        def _():
            for c in xchunks(i, 128):
                w3_chunk(wqb_hbm, wqb_v, S_WQB, c, 0)
                w3_chunk(wuk_hbm, wuk_v, S_WUK, c, 1)

        @pl.when(jnp.logical_and(i >= IT_CKV0, i < IT_W20))
        def _():
            for c in xchunks(i - IT_CKV0, 256):
                rows = pl.ds(pl.multiple_of(c * 32, 32), 32)
                for bb in range(NB):
                    pltpu.make_async_copy(ckv_hbm.at[bb, rows, :], ckv_v.at[bb, rows, :],
                                          sems.at[S_CKV0 + bb]).start(priority=bb)

        @pl.when(jnp.logical_and(i >= IT_W20, i < IT_WEND))
        def _():
            for c in xchunks(i - IT_W20, 128):
                w3_chunk(wuv_hbm, wuv_v, S_WUV, c, 0)
                rows = pl.ds(pl.multiple_of((c % 4) * 32, 32), 32)
                pltpu.make_async_copy(wob_hbm.at[c // 4, rows, :], wob_v.at[c // 4, rows, :],
                                      sems.at[S_WOB]).start(priority=1)

        b_phases(i)
        return carry

    def b_phases(i):
        @pl.when(i == IT_P1)
        def _():
            pltpu.make_async_copy(xb_hbm, xb_v, sems.at[S_XB]).wait()
            w3_wait(wqb_hbm, wqb_v, S_WQB)
            w3_wait(wuk_hbm, wuk_v, S_WUK)

        @pl.when(jnp.logical_and(i >= IT_P1, i < IT_P1 + H // 2))
        def _():
            b_query_piece(i - IT_P1)

        @pl.when(i == IT_P2)
        def _():
            for bb in range(NB):
                pltpu.make_async_copy(ckv_hbm.at[0], ckv_v.at[0], sems.at[S_CKV0 + bb]).wait()

        @pl.when(jnp.logical_and(i >= IT_P2, i < IT_P2 + NBCH))
        def _():
            for bb in range(NB):
                b_score_piece(bb, i - IT_P2)

        @pl.when(jnp.logical_and(i >= IT_P3, i < IT_P3 + NBCH))
        def _():
            for bb in range(NB):
                b_value_piece(bb, i - IT_P3)

        @pl.when(i == IT_P4)
        def _():
            w3_wait(wuv_hbm, wuv_v, S_WUV)
            pltpu.make_async_copy(wob_hbm, wob_v, sems.at[S_WOB]).wait()
            cl_ref[...] = cl_ref[...] / lb_ref[:, 0:1]

        @pl.when(jnp.logical_and(i >= IT_P4, i < IT_P4 + H // 2))
        def _():
            b_out_piece(i - IT_P4)

    lax.fori_loop(0, NB * H, step, 0)

    for b in range(NB):
        out_ref[b:b + 1, 0:DM] = acca_ref[b, 0:1, :].astype(out_ref.dtype)
        out_ref[b:b + 1, DM:2 * DM] = accb_ref[b:b + 1, :].astype(out_ref.dtype)


@jax.jit
def pallas_concat_heads__gqa_block_cached__compressed_kv_cla__decode_kernel(
    A_x, A_k_cache, A_v_cache, A_wq, A_wo, B_x, B_c_kv, B_w_q, B_w_uk, B_w_uv, B_w_o,
):
    assert A_x.shape == (NB, 1, DM) and B_x.shape == (NB, 1, DM)
    assert A_k_cache.shape == (NB, H, SK, DH) and A_v_cache.shape == (NB, H, SK, DH)
    assert B_c_kv.shape == (NB, SK, DC)
    bf16, f32, u32 = jnp.bfloat16, jnp.float32, jnp.uint32
    any_spec = pl.BlockSpec(memory_space=pl.ANY)
    out = pl.pallas_call(
        _kernel,
        out_shape=jax.ShapeDtypeStruct((NB, 2 * DM), bf16),
        in_specs=[any_spec] * 11,
        out_specs=pl.BlockSpec(memory_space=pltpu.VMEM),
        scratch_shapes=[
            pltpu.VMEM((NB, DM), bf16),
            pltpu.VMEM((NB, DM), bf16),
            pltpu.VMEM((R, SK // 2, DH), u32),
            pltpu.VMEM((R, SK // 2, DH), u32),
            pltpu.VMEM((DM, H * DH), bf16),
            pltpu.VMEM((H * DH, DM), bf16),
            pltpu.VMEM((NB, SK, DC), bf16),
            pltpu.VMEM((DM * H // 2, DH), u32),
            pltpu.VMEM((DC * H // 2, DH), u32),
            pltpu.VMEM((DC * H // 2, DH), u32),
            pltpu.VMEM((H, DH, DM), bf16),
            pltpu.VMEM((NB * H, DH), f32),
            pltpu.VMEM((NB, 8, DM), f32),
            pltpu.VMEM((NB * H, DC), f32),
            pltpu.VMEM((NB * H, SK), f32),
            pltpu.VMEM((NB * H, 128), f32),
            pltpu.VMEM((NB * H, 128), f32),
            pltpu.VMEM((NB * H, DC), f32),
            pltpu.VMEM((8, DM), f32),
            pltpu.SemaphoreType.DMA((NSEM,)),
        ],
        compiler_params=pltpu.CompilerParams(vmem_limit_bytes=100 * 1024 * 1024,
                                             disable_bounds_checks=True),
    )(A_x.reshape(NB, DM), A_k_cache, A_v_cache, A_wq, A_wo,
      B_x.reshape(NB, DM), B_c_kv, B_w_q, B_w_uk, B_w_uv, B_w_o)
    return out.reshape(NB, 1, 2 * DM)
```

```python
import math

import jax
import jax.numpy as jnp
from jax import lax
import jax.experimental.pallas as pl
import jax.experimental.pallas.tpu as pltpu

NB = 2
H = 32
SK = 8192
DH = 128
DM = 512
DC = 512
NHEAD = NB * H

R = 3
LOOK = 2
NSTR = 4
KV_UNITS = 64
KR = 64
QU = KV_UNITS // NSTR
QR = QU * KR

XPI = 16
IT_CKV0 = 128 // XPI
IT_W20 = IT_CKV0 + 256 // XPI
IT_WEND = IT_W20 + 128 // XPI

BCH = 1024
NBCH = SK // BCH
NPAIR = H // 2
IT_P1 = IT_CKV0 + 1
IT_P2 = max(IT_P1 + NPAIR, IT_W20 + 1)
IT_P3 = IT_P2 + NBCH
IT_P4 = max(IT_P3 + NBCH, IT_WEND + 1)
assert IT_P4 + NPAIR <= NHEAD - 1

S_XA, S_XB, S_WQA, S_WOA, S_WQB, S_WUK, S_WUV, S_WOB = range(8)
S_CKV = 8
S_K = S_CKV + NB
S_V = S_K + R
S_VL = S_V + R
NSEM = S_VL + NSTR

SC2 = DH ** -0.5 * math.log2(math.e)


def _round_robin(n, nstr):
    per = n // nstr
    return [s * per + j for j in range(per) for s in range(nstr)]


def _rows2(r0, r1, n):
    shape = (n, r0.shape[-1])
    row = lax.broadcasted_iota(jnp.int32, shape, 0)
    return jnp.where(row == 0, jnp.broadcast_to(r0, shape),
                     jnp.where(row == 1, jnp.broadcast_to(r1, shape), 0.0))


def _split_pair(w):
    lo = lax.bitcast_convert_type(w << 16, jnp.float32)
    hi = lax.bitcast_convert_type(w & jnp.uint32(0xFFFF0000), jnp.float32)
    return lo.astype(jnp.bfloat16), hi.astype(jnp.bfloat16)


def _kernel(xa_hbm, k_hbm, v_hbm, wqa_hbm, woa_hbm,
            xb_hbm, ckv_hbm, wqb_hbm, wuk_hbm, wuv_hbm, wob_hbm,
            out_ref,
            xa_v, xb_v, kbuf, vbuf, wqa_v, woa_v, ckv_v, wqb_v, wuk_v, wuv_v, wob_v,
            qa_ref, acca_ref, ql_ref, sb_ref, mb_ref, lb_ref, cl_ref, accb_ref, sems):
    u32, f32, bf16 = jnp.uint32, jnp.float32, jnp.bfloat16
    nt = (((1,), (1,)), ((), ()))

    def wait_all(buf, sem):
        pltpu.make_async_copy(buf, buf, sems.at[sem]).wait()

    k32 = k_hbm.bitcast(u32)
    v32 = v_hbm.bitcast(u32)

    def kv_piece(src, buf, i, unit, sem, prio):
        rows = pl.ds(unit * KR, KR)
        pltpu.make_async_copy(src.at[i // H, i % H, rows, :], buf.at[i % R, rows, :],
                              sems.at[sem]).start(priority=prio)

    def kv_start(i, part=0, nparts=1):
        units = _round_robin(KV_UNITS, NSTR)
        for u in units[len(units) * part // nparts:len(units) * (part + 1) // nparts]:
            kv_piece(k32, kbuf, i, u, S_K + i % R, 0)
            kv_piece(v32, vbuf, i, u, S_V + i % R, 1)

    def kv_start_last(i):
        vunits = [(s, s * QU + u) for s in range(NSTR) for u in _round_robin(QU, 2)]
        half = KV_UNITS // 2
        for j, u in enumerate(_round_robin(KV_UNITS, NSTR)):
            kv_piece(k32, kbuf, i, u, S_K + i % R, 0)
            if j % 2 == 0:
                s, uv = vunits[j // 2]
                kv_piece(v32, vbuf, i, uv, S_VL + s, 1)
        for j, (s, uv) in enumerate(vunits[half:]):
            kv_piece(v32, vbuf, i, uv, S_VL + s, j % 2)

    def w3_piece(w_hbm, w_v, sem, unit, prio):
        rows = pl.ds(unit * 4, 4)
        pltpu.make_async_copy(w_hbm.bitcast(u32).at[rows],
                              w_v.reshape(DM, NPAIR, DH).at[rows],
                              sems.at[sem]).start(priority=prio)

    def rows_piece(src, dst, sem, unit, prio):
        rows = pl.ds(pl.multiple_of(unit * 32, 32), 32)
        pltpu.make_async_copy(src.at[rows, :], dst.at[rows, :],
                              sems.at[sem]).start(priority=prio)

    def extra_units(it, total):
        per, n = total // NSTR, XPI // NSTR
        return [s * per + it * n + j for j in range(n) for s in range(NSTR)]

    wob2_hbm = wob_hbm.reshape(H * DH, DM)

    def extras_start(i):
        @pl.when(i < IT_CKV0)
        def _():
            for u in extra_units(i, 128):
                w3_piece(wqb_hbm, wqb_v, S_WQB, u, 0)
                w3_piece(wuk_hbm, wuk_v, S_WUK, u, 1)

        @pl.when(jnp.logical_and(i >= IT_CKV0, i < IT_W20))
        def _():
            for u in extra_units(i - IT_CKV0, 256):
                for b in range(NB):
                    rows_piece(ckv_hbm.at[b], ckv_v.at[b], S_CKV + b, u, b)

        @pl.when(jnp.logical_and(i >= IT_W20, i < IT_WEND))
        def _():
            for u in extra_units(i - IT_W20, 128):
                w3_piece(wuv_hbm, wuv_v, S_WUV, u, 0)
                rows_piece(wob2_hbm, wob_v, S_WOB, u, 1)

    pltpu.make_async_copy(xa_hbm, xa_v, sems.at[S_XA]).start(priority=0)
    pltpu.make_async_copy(xb_hbm, xb_v, sems.at[S_XB]).start(priority=1)
    for u in _round_robin(128, NSTR):
        rs, cs = pl.ds(u // 2 * 8, 8), pl.ds(u % 2 * 2048, 2048)
        pltpu.make_async_copy(wqa_hbm.at[rs, cs], wqa_v.at[rs, cs],
                              sems.at[S_WQA]).start(priority=0)
        rows_piece(woa_hbm, woa_v, S_WOA, u, 1)
    kv_start(0)

    wait_all(xa_v, S_XA)
    wait_all(wqa_v, S_WQA)
    xa = xa_v[...].astype(f32)
    xa = _rows2(xa[0:1], xa[1:2], 16).astype(bf16)
    qa = jnp.dot(xa, wqa_v[...], preferred_element_type=f32)
    qa = qa.astype(bf16).astype(f32)
    for b in range(NB):
        for h in range(H):
            qa_ref[pl.ds(b * H + h, 1), :] = qa[b:b + 1, h * DH:(h + 1) * DH]

    kv_start(1)

    acca_ref[...] = jnp.zeros(acca_ref.shape, f32)
    accb_ref[...] = jnp.zeros(accb_ref.shape, f32)
    mb_ref[...] = jnp.full(mb_ref.shape, -jnp.inf, f32)
    lb_ref[...] = jnp.zeros(lb_ref.shape, f32)
    cl_ref[...] = jnp.zeros(cl_ref.shape, f32)
    wait_all(woa_v, S_WOA)

    def issue_part(i, part):
        @pl.when(i + LOOK < NHEAD - 1)
        def _():
            kv_start(i + LOOK, part, 3)

    def a_head(i, last=False):
        slot = i % R
        wait_all(kbuf.at[slot], S_K + slot)
        q = jnp.broadcast_to(qa_ref[pl.ds(i, 1), :], (8, DH)).astype(bf16)
        kk = pltpu.bitcast(kbuf[slot], bf16)
        s = lax.dot_general(q, kk, nt, preferred_element_type=f32)
        m = jnp.max(s, axis=-1, keepdims=True)
        p = jnp.exp2((s - m) * SC2)
        l = jnp.sum(p, axis=-1, keepdims=True)
        p = p.astype(bf16)
        if not last:
            issue_part(i, 0)
            wait_all(vbuf.at[slot], S_V + slot)
            o = jnp.dot(p, pltpu.bitcast(vbuf[slot], bf16), preferred_element_type=f32)
        else:
            o = jnp.zeros((8, DH), f32)
            for sq in range(NSTR):
                rows = pl.ds(sq * QR, QR)
                wait_all(vbuf.at[slot, rows, :], S_VL + sq)
                o = o + jnp.dot(p[:, sq * 2 * QR:(sq + 1) * 2 * QR],
                                pltpu.bitcast(vbuf[slot, rows, :], bf16),
                                preferred_element_type=f32)
        o = (o / l).astype(bf16)
        w0 = pl.multiple_of((i % H) * DH, DH)
        acca_ref[i // H] += jnp.dot(o, woa_v[pl.ds(w0, DH), :], preferred_element_type=f32)

    def b_query_piece(j):
        xb = xb_v[...].astype(f32)
        xb = _rows2(xb[0:1], xb[1:2], 16).astype(bf16)
        wq2 = _split_pair(wqb_v[pl.ds(j, DM, stride=NPAIR), :])
        wk2 = _split_pair(wuk_v[pl.ds(j, DC, stride=NPAIR), :])
        for hh in range(2):
            h = 2 * j + hh
            q = jnp.dot(xb, wq2[hh], preferred_element_type=f32)
            ql = lax.dot_general(q.astype(bf16), wk2[hh], nt, preferred_element_type=f32)
            ql_ref[pl.ds(h, 1), :] = ql[0:1, :]
            ql_ref[pl.ds(H + h, 1), :] = ql[1:2, :]

    def b_score_piece(b, j):
        rows = slice(b * H, (b + 1) * H)
        keys = pl.ds(pl.multiple_of(j * BCH, BCH), BCH)
        s = lax.dot_general(ql_ref[rows, :].astype(bf16), ckv_v[b, keys, :], nt,
                            preferred_element_type=f32)
        sb_ref[rows, keys] = s
        mb_ref[rows, :] = jnp.maximum(mb_ref[rows, :], jnp.max(s, axis=-1, keepdims=True))

    def b_value_piece(b, j):
        rows = slice(b * H, (b + 1) * H)
        keys = pl.ds(pl.multiple_of(j * BCH, BCH), BCH)
        p = jnp.exp2((sb_ref[rows, keys] - mb_ref[rows, 0:1]) * SC2)
        lb_ref[rows, :] += jnp.sum(p, axis=-1, keepdims=True)
        cl_ref[rows, :] += jnp.dot(p.astype(bf16), ckv_v[b, keys, :],
                                   preferred_element_type=f32)

    def b_out_piece(j):
        wv2 = _split_pair(wuv_v[pl.ds(j, DC, stride=NPAIR), :])
        acc = accb_ref[...]
        for hh in range(2):
            h = 2 * j + hh
            cl = _rows2(cl_ref[pl.ds(h, 1), :], cl_ref[pl.ds(H + h, 1), :], 16)
            ctx = jnp.dot(cl.astype(bf16), wv2[hh], preferred_element_type=f32)
            w0 = pl.multiple_of(h * DH, DH)
            acc = acc + jnp.dot(ctx.astype(bf16), wob_v[pl.ds(w0, DH), :],
                                preferred_element_type=f32)[0:8]
        accb_ref[...] = acc

    def b_pieces(i):
        @pl.when(i == IT_P1)
        def _():
            wait_all(xb_v, S_XB)
            wait_all(wqb_v, S_WQB)
            wait_all(wuk_v, S_WUK)

        @pl.when(jnp.logical_and(i >= IT_P1, i < IT_P1 + NPAIR))
        def _():
            b_query_piece(i - IT_P1)

        @pl.when(i == IT_P2)
        def _():
            for b in range(NB):
                wait_all(ckv_v.at[b], S_CKV + b)

        @pl.when(jnp.logical_and(i >= IT_P2, i < IT_P2 + NBCH))
        def _():
            for b in range(NB):
                b_score_piece(b, i - IT_P2)

        @pl.when(jnp.logical_and(i >= IT_P3, i < IT_P3 + NBCH))
        def _():
            for b in range(NB):
                b_value_piece(b, i - IT_P3)

        @pl.when(i == IT_P4)
        def _():
            wait_all(wuv_v, S_WUV)
            wait_all(wob_v, S_WOB)
            cl_ref[...] = cl_ref[...] / lb_ref[:, 0:1]

        @pl.when(jnp.logical_and(i >= IT_P4, i < IT_P4 + NPAIR))
        def _():
            b_out_piece(i - IT_P4)

    def step(i, carry):
        a_head(i)
        issue_part(i, 1)

        @pl.when(i + LOOK == NHEAD - 1)
        def _():
            kv_start_last(i + LOOK)

        extras_start(i)
        b_pieces(i)
        issue_part(i, 2)
        return carry

    lax.fori_loop(0, NHEAD - 1, step, 0)
    a_head(NHEAD - 1, last=True)

    for b in range(NB):
        out_ref[b:b + 1, 0:DM] = acca_ref[b, 0:1, :].astype(out_ref.dtype)
        out_ref[b:b + 1, DM:2 * DM] = accb_ref[b:b + 1, :].astype(out_ref.dtype)


@jax.jit
def pallas_concat_heads__gqa_block_cached__compressed_kv_cla__decode_kernel(
    A_x: jax.Array,
    A_k_cache: jax.Array,
    A_v_cache: jax.Array,
    A_wq: jax.Array,
    A_wo: jax.Array,
    B_x: jax.Array,
    B_c_kv: jax.Array,
    B_w_q: jax.Array,
    B_w_uk: jax.Array,
    B_w_uv: jax.Array,
    B_w_o: jax.Array,
):
    assert A_x.shape == (NB, 1, DM) and B_x.shape == (NB, 1, DM)
    assert A_k_cache.shape == (NB, H, SK, DH) and A_v_cache.shape == (NB, H, SK, DH)
    assert A_wq.shape == (DM, H * DH) and A_wo.shape == (H * DH, DM)
    assert B_c_kv.shape == (NB, SK, DC)
    assert B_w_q.shape == (DM, H, DH) and B_w_o.shape == (H, DH, DM)
    assert B_w_uk.shape == (DC, H, DH) and B_w_uv.shape == (DC, H, DH)
    bf16, f32, u32 = jnp.bfloat16, jnp.float32, jnp.uint32
    out = pl.pallas_call(
        _kernel,
        out_shape=jax.ShapeDtypeStruct((NB, 2 * DM), bf16),
        in_specs=[pl.BlockSpec(memory_space=pl.ANY)] * 11,
        out_specs=pl.BlockSpec(memory_space=pltpu.VMEM),
        scratch_shapes=[
            pltpu.VMEM((NB, DM), bf16),
            pltpu.VMEM((NB, DM), bf16),
            pltpu.VMEM((R, SK // 2, DH), u32),
            pltpu.VMEM((R, SK // 2, DH), u32),
            pltpu.VMEM((DM, H * DH), bf16),
            pltpu.VMEM((H * DH, DM), bf16),
            pltpu.VMEM((NB, SK, DC), bf16),
            pltpu.VMEM((DM * NPAIR, DH), u32),
            pltpu.VMEM((DC * NPAIR, DH), u32),
            pltpu.VMEM((DC * NPAIR, DH), u32),
            pltpu.VMEM((H * DH, DM), bf16),
            pltpu.VMEM((NHEAD, DH), f32),
            pltpu.VMEM((NB, 8, DM), f32),
            pltpu.VMEM((NHEAD, DC), f32),
            pltpu.VMEM((NHEAD, SK), f32),
            pltpu.VMEM((NHEAD, 128), f32),
            pltpu.VMEM((NHEAD, 128), f32),
            pltpu.VMEM((NHEAD, DC), f32),
            pltpu.VMEM((8, DM), f32),
            pltpu.SemaphoreType.DMA((NSEM,)),
        ],
        compiler_params=pltpu.CompilerParams(vmem_limit_bytes=100 * 1024 * 1024),
    )(A_x.reshape(NB, DM), A_k_cache, A_v_cache, A_wq, A_wo,
      B_x.reshape(NB, DM), B_c_kv, B_w_q, B_w_uk, B_w_uv, B_w_o)
    return out.reshape(NB, 1, 2 * DM)
```

```python
import math

import numpy as np
import jax
import jax.numpy as jnp
from jax import lax
import jax.experimental.pallas as pl
import jax.experimental.pallas.tpu as pltpu

NB = 2
H = 32
SK = 8192
DH = 128
DM = 512
DC = 512
NHEAD = NB * H

R = 3
LOOK = 2
NSTR = 4
KV_UNITS = 64
KR = 128
QU = KV_UNITS // NSTR
QR = QU * KR

XPI = 16
IT_CKV0 = 128 // XPI
IT_W20 = IT_CKV0 + 256 // XPI
IT_WEND = IT_W20 + 128 // XPI

BCH = 1024
NBCH = SK // BCH
NPAIR = H // 2
NCV = 4
IT_C1 = IT_CKV0 + 1
IT_P1 = IT_C1 + NCV
IT_P2 = max(IT_P1 + NPAIR, IT_W20 + 1)
IT_P3 = IT_P2 + NBCH
IT_C2 = max(IT_P3 + NBCH, IT_WEND + 1)
IT_P4 = IT_C2 + NCV
assert IT_P4 + NPAIR // 2 <= NHEAD - 1

S_XA, S_XB, S_WQA, S_WOA, S_WQB, S_WUK, S_WUV, S_WOB = range(8)
S_CKV = 8
S_K = S_CKV + NB
S_V = S_K + R
S_VL = S_V + R
NSEM = S_VL + NSTR

SC2 = DH ** -0.5 * math.log2(math.e)


def _round_robin(n, nstr):
    per = n // nstr
    return [s * per + j for j in range(per) for s in range(nstr)]


def _rows2(r0, r1, n):
    shape = (n, r0.shape[-1])
    row = lax.broadcasted_iota(jnp.int32, shape, 0)
    return jnp.where(row == 0, jnp.broadcast_to(r0, shape),
                     jnp.where(row == 1, jnp.broadcast_to(r1, shape), 0.0))


def _split_pair(w):
    lo = lax.bitcast_convert_type(w << 16, jnp.float32)
    hi = lax.bitcast_convert_type(w & np.uint32(0xFFFF0000), jnp.float32)
    return lo.astype(jnp.bfloat16), hi.astype(jnp.bfloat16)


def _kernel(xa_hbm, k_hbm, v_hbm, wqa_hbm, woa_hbm,
            xb_hbm, ckv_hbm, wqb_hbm, wuk_hbm, wuv_hbm, wob_hbm,
            out_ref,
            xa_v, xb_v, kbuf, vbuf, wqa_v, woa_v, ckv_v, wqb_s, wuk_s, wuv_s, wob_v,
            wqb_v, wuk_v, wuv_v,
            qa_ref, acca_ref, ql_ref, sb_ref, mb_ref, lb_ref, cl_ref, accb_ref, sems):
    u32, f32, bf16 = jnp.uint32, jnp.float32, jnp.bfloat16
    nt = (((1,), (1,)), ((), ()))

    def wait_all(buf, sem):
        pltpu.make_async_copy(buf, buf, sems.at[sem]).wait()

    def kv_piece(src, buf, i, unit, sem, prio):
        rows = pl.ds(unit * KR, KR)
        pltpu.make_async_copy(src.at[i // H, i % H, rows, :], buf.at[i % R, rows, :],
                              sems.at[sem]).start(priority=prio)

    def kv_start(i, part=0, nparts=1):
        units = _round_robin(KV_UNITS, NSTR)
        for u in units[len(units) * part // nparts:len(units) * (part + 1) // nparts]:
            kv_piece(k_hbm, kbuf, i, u, S_K + i % R, 0)
            kv_piece(v_hbm, vbuf, i, u, S_V + i % R, 1)

    def kv_start_last(i):
        vunits = [(s, s * QU + u) for s in range(NSTR) for u in _round_robin(QU, 2)]
        half = KV_UNITS // 2
        for j, u in enumerate(_round_robin(KV_UNITS, NSTR)):
            kv_piece(k_hbm, kbuf, i, u, S_K + i % R, 0)
            if j % 2 == 0:
                s, uv = vunits[j // 2]
                kv_piece(v_hbm, vbuf, i, uv, S_VL + s, 1)
        for j, (s, uv) in enumerate(vunits[half:]):
            kv_piece(v_hbm, vbuf, i, uv, S_VL + s, j % 2)

    def w3_piece(w_hbm, w_s, sem, unit, prio):
        rows = pl.ds(unit * 4, 4)
        pltpu.make_async_copy(w_hbm.at[rows], w_s.at[rows], sems.at[sem]).start(priority=prio)

    def rows_piece(src, dst, sem, unit, prio):
        rows = pl.ds(pl.multiple_of(unit * 32, 32), 32)
        pltpu.make_async_copy(src.at[rows, :], dst.at[rows, :],
                              sems.at[sem]).start(priority=prio)

    def extra_units(it, total):
        per, n = total // NSTR, XPI // NSTR
        return [s * per + it * n + j for j in range(n) for s in range(NSTR)]

    def extras_start(i):
        @pl.when(i < IT_CKV0)
        def _():
            for u in extra_units(i, 128):
                w3_piece(wqb_hbm, wqb_s, S_WQB, u, 0)
                w3_piece(wuk_hbm, wuk_s, S_WUK, u, 1)

        @pl.when(jnp.logical_and(i >= IT_CKV0, i < IT_W20))
        def _():
            for u in extra_units(i - IT_CKV0, 256):
                for b in range(NB):
                    rows_piece(ckv_hbm.at[b], ckv_v.at[b], S_CKV + b, u, b)

        @pl.when(jnp.logical_and(i >= IT_W20, i < IT_WEND))
        def _():
            for u in extra_units(i - IT_W20, 128):
                w3_piece(wuv_hbm, wuv_s, S_WUV, u, 0)
                rows_piece(wob_hbm.at[u // 4], wob_v.at[u // 4], S_WOB, u % 4, 1)

    pltpu.make_async_copy(xa_hbm, xa_v, sems.at[S_XA]).start(priority=0)
    pltpu.make_async_copy(xb_hbm, xb_v, sems.at[S_XB]).start(priority=1)
    for u in _round_robin(128, NSTR):
        rs, cs = pl.ds(u // 2 * 8, 8), pl.ds(u % 2 * 2048, 2048)
        pltpu.make_async_copy(wqa_hbm.at[rs, cs], wqa_v.at[rs, cs],
                              sems.at[S_WQA]).start(priority=0)
        rows_piece(woa_hbm, woa_v, S_WOA, u, 1)
    kv_start(0)

    wait_all(xa_v, S_XA)
    wait_all(wqa_v, S_WQA)
    xa = xa_v[...].astype(f32)
    xa = _rows2(xa[0:1], xa[1:2], 16).astype(bf16)
    qa = jnp.dot(xa, wqa_v[...], preferred_element_type=f32)
    qa = qa.astype(bf16).astype(f32)
    for b in range(NB):
        for h in range(H):
            qa_ref[pl.ds(b * H + h, 1), :] = qa[b:b + 1, h * DH:(h + 1) * DH]

    kv_start(1)

    acca_ref[...] = jnp.zeros(acca_ref.shape, f32)
    accb_ref[...] = jnp.zeros(accb_ref.shape, f32)
    mb_ref[...] = jnp.full(mb_ref.shape, -jnp.inf, f32)
    lb_ref[...] = jnp.zeros(lb_ref.shape, f32)
    cl_ref[...] = jnp.zeros(cl_ref.shape, f32)
    wait_all(woa_v, S_WOA)

    def issue_part(i, part):
        @pl.when(i + LOOK < NHEAD - 1)
        def _():
            kv_start(i + LOOK, part, 3)

    def a_head(i, last=False):
        slot = i % R
        wait_all(kbuf.at[slot], S_K + slot)
        q = jnp.broadcast_to(qa_ref[pl.ds(i, 1), :], (8, DH)).astype(bf16)
        s = lax.dot_general(q, kbuf[slot], nt, preferred_element_type=f32)
        m = jnp.max(s, axis=-1, keepdims=True)
        p = jnp.exp2((s - m) * SC2)
        l = jnp.sum(p, axis=-1, keepdims=True)
        p = p.astype(bf16)
        if not last:
            issue_part(i, 0)
            wait_all(vbuf.at[slot], S_V + slot)
            o = jnp.dot(p, vbuf[slot], preferred_element_type=f32)
        else:
            o = jnp.zeros((8, DH), f32)
            for sq in range(NSTR):
                rows = pl.ds(sq * QR, QR)
                wait_all(vbuf.at[slot, rows, :], S_VL + sq)
                o = o + jnp.dot(p[:, sq * QR:(sq + 1) * QR], vbuf[slot, rows, :],
                                preferred_element_type=f32)
        o = (o / l).astype(bf16)
        w0 = pl.multiple_of((i % H) * DH, DH)
        acca_ref[i // H] += jnp.dot(o, woa_v[pl.ds(w0, DH), :], preferred_element_type=f32)

    def repack_piece(w_s, w_v, c):
        n = DM // NCV
        w = w_s[pl.ds(pl.multiple_of(c * n, n), n)].reshape(n * H, DH)
        w_v[pl.ds(pl.multiple_of(c * n * NPAIR, n * NPAIR), n * NPAIR), :] = pltpu.bitcast(w, u32)

    def b_query_piece(j):
        xb = xb_v[...].astype(f32)
        xb = _rows2(xb[0:1], xb[1:2], 16).astype(bf16)
        wq2 = _split_pair(wqb_v[pl.ds(j, DM, stride=NPAIR), :])
        wk2 = _split_pair(wuk_v[pl.ds(j, DC, stride=NPAIR), :])
        for hh in range(2):
            h = 2 * j + hh
            q = jnp.dot(xb, wq2[hh], preferred_element_type=f32)
            ql = lax.dot_general(q.astype(bf16), wk2[hh], nt, preferred_element_type=f32)
            ql_ref[pl.ds(h, 1), :] = ql[0:1, :]
            ql_ref[pl.ds(H + h, 1), :] = ql[1:2, :]

    def b_score_piece(b, j):
        rows = slice(b * H, (b + 1) * H)
        keys = pl.ds(pl.multiple_of(j * BCH, BCH), BCH)
        s = lax.dot_general(ql_ref[rows, :].astype(bf16), ckv_v[b, keys, :], nt,
                            preferred_element_type=f32)
        sb_ref[rows, keys] = s
        mb_ref[rows, :] = jnp.maximum(mb_ref[rows, :], jnp.max(s, axis=-1, keepdims=True))

    def b_value_piece(b, j):
        rows = slice(b * H, (b + 1) * H)
        keys = pl.ds(pl.multiple_of(j * BCH, BCH), BCH)
        p = jnp.exp2((sb_ref[rows, keys] - mb_ref[rows, 0:1]) * SC2)
        lb_ref[rows, :] += jnp.sum(p, axis=-1, keepdims=True)
        cl_ref[rows, :] += jnp.dot(p.astype(bf16), ckv_v[b, keys, :],
                                   preferred_element_type=f32)

    def b_out_piece(j):
        wv2 = _split_pair(wuv_v[pl.ds(j, DC, stride=NPAIR), :])
        acc = accb_ref[...]
        for hh in range(2):
            h = 2 * j + hh
            cl = _rows2(cl_ref[pl.ds(h, 1), :], cl_ref[pl.ds(H + h, 1), :], 16)
            ctx = jnp.dot(cl.astype(bf16), wv2[hh], preferred_element_type=f32)
            acc = acc + jnp.dot(ctx.astype(bf16), wob_v[h],
                                preferred_element_type=f32)[0:8]
        accb_ref[...] = acc

    def b_pieces(i):
        @pl.when(i == IT_C1)
        def _():
            wait_all(xb_v, S_XB)
            wait_all(wqb_s, S_WQB)
            wait_all(wuk_s, S_WUK)

        @pl.when(jnp.logical_and(i >= IT_C1, i < IT_C1 + NCV))
        def _():
            repack_piece(wqb_s, wqb_v, i - IT_C1)
            repack_piece(wuk_s, wuk_v, i - IT_C1)

        @pl.when(jnp.logical_and(i >= IT_P1, i < IT_P1 + NPAIR))
        def _():
            b_query_piece(i - IT_P1)

        @pl.when(i == IT_P2)
        def _():
            for b in range(NB):
                wait_all(ckv_v.at[b], S_CKV + b)

        @pl.when(jnp.logical_and(i >= IT_P2, i < IT_P2 + NBCH))
        def _():
            for b in range(NB):
                b_score_piece(b, i - IT_P2)

        @pl.when(jnp.logical_and(i >= IT_P3, i < IT_P3 + NBCH))
        def _():
            for b in range(NB):
                b_value_piece(b, i - IT_P3)

        @pl.when(i == IT_C2)
        def _():
            wait_all(wuv_s, S_WUV)
            wait_all(wob_v, S_WOB)
            cl_ref[...] = cl_ref[...] / lb_ref[:, 0:1]

        @pl.when(jnp.logical_and(i >= IT_C2, i < IT_C2 + NCV))
        def _():
            repack_piece(wuv_s, wuv_v, i - IT_C2)

        @pl.when(jnp.logical_and(i >= IT_P4, i < IT_P4 + NPAIR // 2))
        def _():
            for jj in range(2):
                b_out_piece(2 * (i - IT_P4) + jj)

    def step(i, carry):
        a_head(i)
        issue_part(i, 1)

        @pl.when(i + LOOK == NHEAD - 1)
        def _():
            kv_start_last(i + LOOK)

        extras_start(i)
        b_pieces(i)
        issue_part(i, 2)
        return carry

    lax.fori_loop(0, NHEAD - 1, step, 0)
    a_head(NHEAD - 1, last=True)

    for b in range(NB):
        out_ref[b:b + 1, 0:DM] = acca_ref[b, 0:1, :].astype(out_ref.dtype)
        out_ref[b:b + 1, DM:2 * DM] = accb_ref[b:b + 1, :].astype(out_ref.dtype)


@jax.jit
def pallas_concat_heads__gqa_block_cached__compressed_kv_cla__decode_kernel(
    A_x: jax.Array,
    A_k_cache: jax.Array,
    A_v_cache: jax.Array,
    A_wq: jax.Array,
    A_wo: jax.Array,
    B_x: jax.Array,
    B_c_kv: jax.Array,
    B_w_q: jax.Array,
    B_w_uk: jax.Array,
    B_w_uv: jax.Array,
    B_w_o: jax.Array,
):
    assert A_x.shape == (NB, 1, DM) and B_x.shape == (NB, 1, DM)
    assert A_k_cache.shape == (NB, H, SK, DH) and A_v_cache.shape == (NB, H, SK, DH)
    assert A_wq.shape == (DM, H * DH) and A_wo.shape == (H * DH, DM)
    assert B_c_kv.shape == (NB, SK, DC)
    assert B_w_q.shape == (DM, H, DH) and B_w_o.shape == (H, DH, DM)
    assert B_w_uk.shape == (DC, H, DH) and B_w_uv.shape == (DC, H, DH)
    bf16, f32, u32 = jnp.bfloat16, jnp.float32, jnp.uint32
    out = pl.pallas_call(
        _kernel,
        out_shape=jax.ShapeDtypeStruct((NB, 2 * DM), bf16),
        in_specs=[pl.BlockSpec(memory_space=pl.ANY)] * 11,
        out_specs=pl.BlockSpec(memory_space=pltpu.VMEM),
        scratch_shapes=[
            pltpu.VMEM((NB, DM), bf16),
            pltpu.VMEM((NB, DM), bf16),
            pltpu.VMEM((R, SK, DH), bf16),
            pltpu.VMEM((R, SK, DH), bf16),
            pltpu.VMEM((DM, H * DH), bf16),
            pltpu.VMEM((H * DH, DM), bf16),
            pltpu.VMEM((NB, SK, DC), bf16),
            pltpu.VMEM((DM, H, DH), bf16),
            pltpu.VMEM((DC, H, DH), bf16),
            pltpu.VMEM((DC, H, DH), bf16),
            pltpu.VMEM((H, DH, DM), bf16),
            pltpu.VMEM((DM * NPAIR, DH), u32),
            pltpu.VMEM((DC * NPAIR, DH), u32),
            pltpu.VMEM((DC * NPAIR, DH), u32),
            pltpu.VMEM((NHEAD, DH), f32),
            pltpu.VMEM((NB, 8, DM), f32),
            pltpu.VMEM((NHEAD, DC), f32),
            pltpu.VMEM((NHEAD, SK), f32),
            pltpu.VMEM((NHEAD, 128), f32),
            pltpu.VMEM((NHEAD, 128), f32),
            pltpu.VMEM((NHEAD, DC), f32),
            pltpu.VMEM((8, DM), f32),
            pltpu.SemaphoreType.DMA((NSEM,)),
        ],
        compiler_params=pltpu.CompilerParams(vmem_limit_bytes=100 * 1024 * 1024),
    )(A_x.reshape(NB, DM), A_k_cache, A_v_cache, A_wq, A_wo,
      B_x.reshape(NB, DM), B_c_kv, B_w_q, B_w_uk, B_w_uv, B_w_o)
    return out.reshape(NB, 1, 2 * DM)
```
